```python
import jax
import jax.numpy as jnp

def _softmax(x, axis=-1):
    return jax.nn.softmax(x, axis=axis)
def _gelu(x):
    return jax.nn.gelu(x, approximate=True)
def _silu(x):
    return jax.nn.silu(x)
def _sigmoid(x):
    return jax.nn.sigmoid(x)
def _layernorm(x, axis=-1, eps=1e-5):
    m = jnp.mean(x, axis=axis, keepdims=True)
    v = jnp.var(x, axis=axis, keepdims=True)
    return (x - m) / jnp.sqrt(v + eps)
def _scatter_add(tgt, idx, src, axis=0):
    return tgt.at[idx].add(src)
def _segment_sum(src, seg, n):
    return jax.ops.segment_sum(src, seg, n)
class _Rng:
    def __init__(self, key):
        self._k = key
    def _next(self):
        self._k, sub = jax.random.split(self._k)
        return sub
    def normal(self, shape):
        return jax.random.normal(self._next(), shape, dtype=jnp.bfloat16)
    def randint(self, lo, hi, shape):
        return jax.random.randint(self._next(), shape, lo, hi, dtype=jnp.int32)
    def uniform(self, shape, lo=0.0, hi=1.0):
        return jax.random.uniform(self._next(), shape, jnp.bfloat16, lo, hi)
    def permutation(self, n):
        return jax.random.permutation(self._next(), n)


kernel_name = 'gated_mix__sliding_local_dilated__compressed_kv_cla__prompt'

def setup_inputs():
    _rng = _Rng(jax.random.key(int.from_bytes(__import__("os").urandom(4), "little")))
    _w = (lambda a: (lambda t: t.astype(jnp.bfloat16) if jnp.issubdtype(t.dtype, jnp.floating) else t)(jnp.asarray(a)))
    def _A_setup():
        B, S, D = 1, 2048, 576
        return {
            "x": _w((lambda *s: _rng.normal(s) * 0.05)(B, S, D)),
            "wqkv": _w((lambda *s: _rng.normal(s) * 0.05)(D, 3 * D)),
            "wo": _w((lambda *s: _rng.normal(s) * 0.05)(D, D)),
        }
    _A_in = _A_setup()

    def _B_setup():
        B, H, Sq, Sk, D, M = 1, 32, 2048, 2048, 128, 576
        Dc = 4 * D
        return {
            "x": _w((lambda *s: _rng.normal(s) * 0.05)(B, Sq, M)),
            "c_kv": _w((lambda *s: _rng.normal(s) * 0.05)(B, Sk, Dc)),
            "w_q": _w((lambda *s: _rng.normal(s) * 0.05)(M, H, D) * (M ** -0.5)),
            "w_uk": _w((lambda *s: _rng.normal(s) * 0.05)(Dc, H, D) * (Dc ** -0.5)),
            "w_uv": _w((lambda *s: _rng.normal(s) * 0.05)(Dc, H, D) * (Dc ** -0.5)),
            "w_o": _w((lambda *s: _rng.normal(s) * 0.05)(H, D, M) * ((H * D) ** -0.5)),
        }
    _B_in = _B_setup()

    return {
        "A_x": _A_in["x"],
        "A_wqkv": _A_in["wqkv"],
        "A_wo": _A_in["wo"],
        "B_x": _B_in["x"],
        "B_c_kv": _B_in["c_kv"],
        "B_w_q": _B_in["w_q"],
        "B_w_uk": _B_in["w_uk"],
        "B_w_uv": _B_in["w_uv"],
        "B_w_o": _B_in["w_o"],
        "gate_w": _w((lambda *s: _rng.normal(s) * 0.05)(576)),
    }

def reference(A_x, A_wqkv, A_wo, B_x, B_c_kv, B_w_q, B_w_uk, B_w_uv, B_w_o, gate_w):
    def _A_ref(x, wqkv, wo):
        B, S, D = x.shape
        H = 32; Dh = D // H
        W, dil = 8, 2
        qkv = (lambda x, *d: x.transpose(*d))((x @ wqkv).reshape(B, S, 3, H, Dh), 2, 0, 3, 1, 4)
        q, k, v = qkv[0], qkv[1], qkv[2]
        scale = Dh ** -0.5
        pos = jnp.arange(S)
        off = jnp.arange(W) * dil
        idx = pos[:, None] - off[None, :]
        mask = idx >= 0
        idx_c = jnp.where(mask, idx, 0).reshape(-1)
        kg = k[:, :, idx_c, :].reshape(B, H, S, W, Dh)
        vg = v[:, :, idx_c, :].reshape(B, H, S, W, Dh)
        logits = jnp.einsum("bhsd,bhswd->bhsw", q, kg) * scale
        logits = jnp.where(mask[None, None, :, :], logits, -1e9)
        attn = _softmax(logits, axis=-1)
        o = jnp.einsum("bhsw,bhswd->bhsd", attn, vg)
        return (lambda x, *d: x.transpose(*d))(o, 0, 2, 1, 3).reshape(B, S, D) @ wo

    def _B_ref(x, c_kv, w_q, w_uk, w_uv, w_o):
        B, Sq, M = x.shape[0], x.shape[1], x.shape[2]
        Sk = c_kv.shape[1]
        H, D = w_q.shape[1], w_q.shape[2]
        q = jnp.einsum("bqm,mhd->bhqd", x, w_q)
        k = jnp.einsum("bkc,chd->bhkd", c_kv, w_uk)
        v = jnp.einsum("bkc,chd->bhkd", c_kv, w_uv)
        scores = jnp.einsum("bhqd,bhkd->bhqk", q, k) * (D ** -0.5)
        off = Sk - Sq
        qi = jnp.arange(Sq)[:, None]
        kj = jnp.arange(Sk)[None, :]
        cmask = kj <= (qi + off)
        scores = jnp.where(cmask[None, None], scores, -1e9)
        p = _softmax(scores, axis=-1)
        ctx = jnp.einsum("bhqk,bhkd->bhqd", p, v)
        return jnp.einsum("bhqd,hdm->bqm", ctx, w_o)

    x = A_x
    g = _sigmoid((x * gate_w).sum(-1, keepdims=True))
    a = _A_ref(x, A_wqkv, A_wo)
    b = _B_ref(x, B_c_kv, B_w_q, B_w_uk, B_w_uv, B_w_o)
    return g * a + (1 - g) * b
```

```python
import math
import jax
import jax.numpy as jnp
from jax import lax
import jax.experimental.pallas as pl
import jax.experimental.pallas.tpu as pltpu

F32 = jnp.float32
BF16 = jnp.bfloat16
S, DM, NH, DH, DC = 2048, 576, 32, 128, 512
HA, DA, WIN, DIL = 32, 18, 8, 2
DP = 640
PADR = 16
BQ = 256
RA = 256
NT = (((1,), (1,)), ((), ()))


def _dot(a, b):
    return jnp.dot(a, b, preferred_element_type=F32)


def _perm(n_in, off, transposed=False):
    shp = (DP, n_in) if transposed else (n_in, DP)
    src = lax.broadcasted_iota(jnp.int32, shp, 1 if transposed else 0)
    dst = lax.broadcasted_iota(jnp.int32, shp, 0 if transposed else 1)
    d = dst >> 5
    h = dst & 31
    return jnp.where((src == off + h * DA + d) & (d < DA), 1.0, 0.0).astype(BF16)


def _unpack(w):
    lo = lax.bitcast_convert_type(w << 16, F32).astype(BF16)
    hi = lax.bitcast_convert_type(w & jnp.uint32(0xFFFF0000), F32).astype(BF16)
    return lo, hi


def _kernel(x_h, wqkv_h, awo_h, c_h, wq_h, wuk_h, wuv_h, wo_h, gw_h, out_h,
            x_v, wqkv_v, awo_v, c_v, wq_v, wuk_v, wuv_v, wo_v, gw_v,
            wa_p, awo_p, ka, va, oa, q_s, k_s, v_s, ctx, out_v, sems, osem):
    srcs = (x_h.at[0], wqkv_h, gw_h, awo_h, c_h.at[0], wq_h, wuk_h, wuv_h, wo_h)
    dsts = (x_v, wqkv_v, gw_v, awo_v, c_v, wq_v, wuk_v, wuv_v, wo_v)
    cps = [pltpu.make_async_copy(s, d, sems.at[i]) for i, (s, d) in enumerate(zip(srcs, dsts))]
    for cp in cps:
        cp.start()

    cps[1].wait()
    for p, (st, wd) in enumerate(((0, 640), (512, 640), (1152, 576))):
        wa_p[:, p * DP:(p + 1) * DP] = _dot(
            wqkv_v[:, st:st + wd], _perm(wd, p * DM - st)).astype(BF16)
    for t in range(5):
        ka[t, 0:PADR, :] = jnp.zeros((PADR, 128), F32)
        va[t, 0:PADR, :] = jnp.zeros((PADR, 128), F32)
    cps[0].wait()

    def a_body(r, carry):
        r0 = pl.multiple_of(r * RA, RA)
        qkv = _dot(x_v[pl.ds(r0, RA), :], wa_p[...])
        for t in range(5):
            ka[t, pl.ds(r0 + PADR, RA), :] = qkv[:, DP + t * 128:DP + (t + 1) * 128]
            va[t, pl.ds(r0 + PADR, RA), :] = qkv[:, 2 * DP + t * 128:2 * DP + (t + 1) * 128]
        q = qkv[:, :DP] * (DA ** -0.5)
        pos = r0 + lax.broadcasted_iota(jnp.int32, (RA, 128), 0)
        lg = []
        for w in range(WIN):
            st = r0 + PADR - w * DIL
            acc = q[:, 0:128] * ka[0, pl.ds(st, RA), :]
            for t in range(1, 5):
                acc = acc + q[:, t * 128:(t + 1) * 128] * ka[t, pl.ds(st, RA), :]
            acc = acc + pltpu.roll(acc, 64, 1)
            acc = acc + pltpu.roll(acc, 32, 1)
            if w:
                acc = jnp.where(pos >= w * DIL, acc, -1e9)
            lg.append(acc)
        m = lg[0]
        for w in range(1, WIN):
            m = jnp.maximum(m, lg[w])
        e = [jnp.exp(l - m) for l in lg]
        den = e[0]
        for w in range(1, WIN):
            den = den + e[w]
        inv = 1.0 / den
        for t in range(5):
            o = e[0] * va[t, pl.ds(r0 + PADR, RA), :]
            for w in range(1, WIN):
                o = o + e[w] * va[t, pl.ds(r0 + PADR - w * DIL, RA), :]
            oa[pl.ds(r0, RA), t * 128:(t + 1) * 128] = (o * inv).astype(BF16)
        return carry

    lax.fori_loop(0, S // RA, a_body, 0)
    cps[3].wait()
    awo_p[...] = _dot(_perm(DM, 0, True), awo_v[...]).astype(BF16)

    for i in (4, 5, 6, 7):
        cps[i].wait()
    wq_u, wuk_u, wuv_u = (r.bitcast(jnp.uint32) for r in (wq_v, wuk_v, wuv_v))
    qscale = DH ** -0.5 * math.log2(math.e)

    def pair_body(j, carry):
        wq2 = jnp.concatenate(_unpack(wq_u[:, j, :]), axis=1)
        wkv = jnp.concatenate(_unpack(wuk_u[:, j, :]) + _unpack(wuv_u[:, j, :]), axis=1)
        for r in range(S // 512):
            rs = slice(r * 512, (r + 1) * 512)
            q2 = (_dot(x_v[rs, :], wq2) * qscale).astype(BF16)
            kv = _dot(c_v[rs, :], wkv).astype(BF16)
            for a in range(2):
                q_s[a, rs, :] = q2[:, a * 128:(a + 1) * 128]
                k_s[a, rs, :] = kv[:, a * 128:(a + 1) * 128]
                v_s[a, rs, :] = kv[:, 256 + a * 128:256 + (a + 1) * 128]

        def head_body(a, c2):
            tri = (lax.broadcasted_iota(jnp.int32, (BQ, BQ), 1)
                   <= lax.broadcasted_iota(jnp.int32, (BQ, BQ), 0))
            for i in range(S // BQ):
                lo, hi = i * BQ, (i + 1) * BQ
                q = q_s[a, lo:hi, :]
                sd = lax.dot_general(q, k_s[a, lo:hi, :], NT, preferred_element_type=F32)
                sd = jnp.where(tri, sd, -1e9)
                m = jnp.max(sd, axis=1, keepdims=True)
                if i:
                    so = lax.dot_general(q, k_s[a, 0:lo, :], NT, preferred_element_type=F32)
                    m = jnp.maximum(m, jnp.max(so, axis=1, keepdims=True))
                pd = jnp.exp2(sd - m)
                l = jnp.sum(pd, axis=1, keepdims=True)
                o = _dot(pd.astype(BF16), v_s[a, lo:hi, :])
                if i:
                    po = jnp.exp2(so - m)
                    l = l + jnp.sum(po, axis=1, keepdims=True)
                    o = o + _dot(po.astype(BF16), v_s[a, 0:lo, :])
                ctx[2 * j + a, lo:hi, :] = (o * (1.0 / l)).astype(BF16)
            return c2

        lax.fori_loop(0, 2, head_body, 0)
        return carry

    lax.fori_loop(0, NH // 2, pair_body, 0)

    cps[8].wait()
    cps[2].wait()
    RO = 256

    def out_cp(r):
        rs = pl.ds(pl.multiple_of(r * RO, RO), RO)
        return pltpu.make_async_copy(out_v.at[rs, :], out_h.at[0, rs, :], osem.at[r])

    def o_body(r, carry):
        rs = pl.ds(pl.multiple_of(r * RO, RO), RO)
        cc = jnp.concatenate([ctx[h, rs, :] for h in range(NH)], axis=1)
        b = _dot(cc, wo_v[...])
        a = _dot(oa[rs, :], awo_p[...])
        z = jnp.sum(x_v[rs, :].astype(F32) * gw_v[...].astype(F32), axis=1, keepdims=True)
        g = 1.0 / (1.0 + jnp.exp(-z))
        out_v[rs, :] = (g * a + (1.0 - g) * b).astype(BF16)
        out_cp(r).start()
        return carry

    lax.fori_loop(0, S // RO, o_body, 0)
    for r in range(S // RO):
        out_cp(r).wait()


@jax.jit
def pallas_gated_mix__sliding_local_dilated__compressed_kv_cla__prompt_kernel(
    A_x, A_wqkv, A_wo, B_x, B_c_kv, B_w_q, B_w_uk, B_w_uv, B_w_o, gate_w,
):
    del B_x
    args = (A_x, A_wqkv, A_wo, B_c_kv, B_w_q, B_w_uk, B_w_uv,
            B_w_o.reshape(NH * DH, DM), gate_w.reshape(1, DM))
    V = pltpu.VMEM
    scratch = [
        V((S, DM), BF16), V((DM, 3 * DM), BF16), V((DM, DM), BF16), V((S, DC), BF16),
        V((DM, NH, DH), BF16), V((DC, NH, DH), BF16), V((DC, NH, DH), BF16),
        V((NH * DH, DM), BF16), V((1, DM), BF16),
        V((DM, 3 * DP), BF16), V((DP, DM), BF16),
        V((5, S + PADR, 128), F32), V((5, S + PADR, 128), F32), V((S, DP), BF16),
        V((2, S, DH), BF16), V((2, S, DH), BF16), V((2, S, DH), BF16),
        V((NH, S, DH), BF16), V((S, DM), BF16),
        pltpu.SemaphoreType.DMA((9,)), pltpu.SemaphoreType.DMA((8,)),
    ]
    return pl.pallas_call(
        _kernel,
        out_shape=jax.ShapeDtypeStruct((1, S, DM), BF16),
        in_specs=[pl.BlockSpec(memory_space=pl.ANY)] * len(args),
        out_specs=pl.BlockSpec(memory_space=pl.ANY),
        scratch_shapes=scratch,
        compiler_params=pltpu.CompilerParams(vmem_limit_bytes=110 * 1024 * 1024),
    )(*args)
```

```python
import math
import jax
import jax.numpy as jnp
from jax import lax
import jax.experimental.pallas as pl
import jax.experimental.pallas.tpu as pltpu

F32 = jnp.float32
BF16 = jnp.bfloat16
S, DM, NH, DH, DC = 2048, 576, 32, 128, 512
HA, DA, WIN, DIL = 32, 18, 8, 2
DP = 640
PADR = 16
BQ = 256
RA = 256
TN = (((0,), (0,)), ((), ()))
NT = (((1,), (1,)), ((), ()))


def _dot(a, b):
    return jnp.dot(a, b, preferred_element_type=F32)


def _perm(n_in, off, transposed=False):
    shp = (DP, n_in) if transposed else (n_in, DP)
    src = lax.broadcasted_iota(jnp.int32, shp, 1 if transposed else 0)
    dst = lax.broadcasted_iota(jnp.int32, shp, 0 if transposed else 1)
    d = dst >> 5
    h = dst & 31
    return jnp.where((src == off + h * DA + d) & (d < DA), 1.0, 0.0).astype(BF16)


def _unpack(w):
    lo = lax.bitcast_convert_type(w << 16, F32).astype(BF16)
    hi = lax.bitcast_convert_type(w & jnp.uint32(0xFFFF0000), F32).astype(BF16)
    return lo, hi


def _kernel(x_h, wqkv_h, awo_h, c_h, wq_h, wuk_h, wuv_h, wo_h, gw_h, out_h,
            xt_v, wqkv_v, awo_v, c_v, wq_v, wuk_v, wuv_v, wo_v, gw_v,
            x_v, wa_p, awo_p, ka, va, oa, q_s, k_s, v_s, ctx, out_v, sems, osem):
    srcs = (x_h.at[0], wqkv_h, gw_h, awo_h, c_h.at[0], wq_h, wuk_h, wuv_h, wo_h)
    dsts = (xt_v.at[0:DM], wqkv_v, gw_v, awo_v, c_v, wq_v, wuk_v, wuv_v, wo_v)
    cps = [pltpu.make_async_copy(s, d, sems.at[i]) for i, (s, d) in enumerate(zip(srcs, dsts))]
    for cp in cps:
        cp.start()

    cps[1].wait()
    for p, (st, wd) in enumerate(((0, 640), (512, 640), (1152, 576))):
        wa_p[:, p * DP:(p + 1) * DP] = _dot(
            wqkv_v[:, st:st + wd], _perm(wd, p * DM - st)).astype(BF16)
    for t in range(5):
        ka[t, 0:PADR, :] = jnp.zeros((PADR, 128), F32)
        va[t, 0:PADR, :] = jnp.zeros((PADR, 128), F32)
    xt_v[DM:DP, :] = jnp.zeros((DP - DM, S), BF16)
    cps[0].wait()

    def a_body(r, carry):
        r0 = pl.multiple_of(r * RA, RA)
        x_v[pl.ds(r0, RA), :] = xt_v[:, pl.ds(r0, RA)].T
        qkv = _dot(x_v[pl.ds(r0, RA), 0:DM], wa_p[...])
        for t in range(5):
            ka[t, pl.ds(r0 + PADR, RA), :] = qkv[:, DP + t * 128:DP + (t + 1) * 128]
            va[t, pl.ds(r0 + PADR, RA), :] = qkv[:, 2 * DP + t * 128:2 * DP + (t + 1) * 128]
        q = qkv[:, :DP] * (DA ** -0.5)
        pos = r0 + lax.broadcasted_iota(jnp.int32, (RA, 128), 0)
        lg = []
        for w in range(WIN):
            st = r0 + PADR - w * DIL
            acc = q[:, 0:128] * ka[0, pl.ds(st, RA), :]
            for t in range(1, 5):
                acc = acc + q[:, t * 128:(t + 1) * 128] * ka[t, pl.ds(st, RA), :]
            acc = acc + pltpu.roll(acc, 64, 1)
            acc = acc + pltpu.roll(acc, 32, 1)
            if w:
                acc = jnp.where(pos >= w * DIL, acc, -1e9)
            lg.append(acc)
        m = lg[0]
        for w in range(1, WIN):
            m = jnp.maximum(m, lg[w])
        e = [jnp.exp(l - m) for l in lg]
        den = e[0]
        for w in range(1, WIN):
            den = den + e[w]
        inv = 1.0 / den
        for t in range(5):
            o = e[0] * va[t, pl.ds(r0 + PADR, RA), :]
            for w in range(1, WIN):
                o = o + e[w] * va[t, pl.ds(r0 + PADR - w * DIL, RA), :]
            oa[pl.ds(r0, RA), t * 128:(t + 1) * 128] = (o * inv).astype(BF16)
        return carry

    lax.fori_loop(0, S // RA, a_body, 0)
    cps[3].wait()
    awo_p[...] = lax.dot_general(awo_v[...], _perm(DM, 0), TN, preferred_element_type=F32).astype(BF16)

    for i in (4, 5, 6, 7):
        cps[i].wait()
    wq_u, wuk_u, wuv_u = (r.bitcast(jnp.uint32) for r in (wq_v, wuk_v, wuv_v))
    qscale = DH ** -0.5 * math.log2(math.e)

    def pair_body(j, carry):
        wq2 = jnp.concatenate(_unpack(wq_u[:, j, :]), axis=1)
        wkv = jnp.concatenate(_unpack(wuk_u[:, j, :]) + _unpack(wuv_u[:, j, :]), axis=1)
        for r in range(S // 512):
            rs = slice(r * 512, (r + 1) * 512)
            q2 = (_dot(x_v[rs, 0:DM], wq2) * qscale).astype(BF16)
            kv = _dot(c_v[rs, :], wkv).astype(BF16)
            for a in range(2):
                q_s[a, rs, :] = q2[:, a * 128:(a + 1) * 128]
                k_s[a, rs, :] = kv[:, a * 128:(a + 1) * 128]
                v_s[a, rs, :] = kv[:, 256 + a * 128:256 + (a + 1) * 128]

        def head_body(a, c2):
            tri = (lax.broadcasted_iota(jnp.int32, (BQ, BQ), 1)
                   <= lax.broadcasted_iota(jnp.int32, (BQ, BQ), 0))
            for i in range(S // BQ):
                lo, hi = i * BQ, (i + 1) * BQ
                q = q_s[a, lo:hi, :]
                sd = lax.dot_general(q, k_s[a, lo:hi, :], NT, preferred_element_type=F32)
                sd = jnp.where(tri, sd, -1e9)
                m = jnp.max(sd, axis=1, keepdims=True)
                if i:
                    so = lax.dot_general(q, k_s[a, 0:lo, :], NT, preferred_element_type=F32)
                    m = jnp.maximum(m, jnp.max(so, axis=1, keepdims=True))
                pd = jnp.exp2(sd - m)
                l = jnp.sum(pd, axis=1, keepdims=True)
                o = _dot(pd.astype(BF16), v_s[a, lo:hi, :])
                if i:
                    po = jnp.exp2(so - m)
                    l = l + jnp.sum(po, axis=1, keepdims=True)
                    o = o + _dot(po.astype(BF16), v_s[a, 0:lo, :])
                ctx[2 * j + a, lo:hi, :] = (o * (1.0 / l)).astype(BF16)
            return c2

        lax.fori_loop(0, 2, head_body, 0)
        return carry

    lax.fori_loop(0, NH // 2, pair_body, 0)

    cps[8].wait()
    cps[2].wait()
    RO = 256

    def out_cp(r):
        rs = pl.ds(pl.multiple_of(r * RO, RO), RO)
        return pltpu.make_async_copy(out_v.at[:, rs], out_h.at[0, :, rs], osem.at[r])

    def o_body(r, carry):
        rs = pl.ds(pl.multiple_of(r * RO, RO), RO)
        cc = jnp.concatenate([ctx[h, rs, :] for h in range(NH)], axis=1)
        wo = jnp.concatenate([wo_v[h] for h in range(NH)], axis=1)
        b = lax.dot_general(wo, cc, NT, preferred_element_type=F32)
        a = lax.dot_general(awo_p[...], oa[rs, :], NT, preferred_element_type=F32)
        z = _dot(jnp.broadcast_to(gw_v[...], (16, DM)), xt_v[0:DM, rs])[0:1]
        g = 1.0 / (1.0 + jnp.exp(-z))
        out_v[:, rs] = (g * a + (1.0 - g) * b).astype(BF16)
        out_cp(r).start()
        return carry

    lax.fori_loop(0, S // RO, o_body, 0)
    for r in range(S // RO):
        out_cp(r).wait()


@jax.jit
def pallas_gated_mix__sliding_local_dilated__compressed_kv_cla__prompt_kernel(
    A_x, A_wqkv, A_wo, B_x, B_c_kv, B_w_q, B_w_uk, B_w_uv, B_w_o, gate_w,
):
    del B_x
    args = (jnp.swapaxes(A_x, 1, 2), A_wqkv, A_wo, B_c_kv, B_w_q, B_w_uk, B_w_uv,
            jnp.swapaxes(B_w_o, 1, 2), gate_w.reshape(1, DM))
    V = pltpu.VMEM
    scratch = [
        V((DP, S), BF16), V((DM, 3 * DM), BF16), V((DM, DM), BF16), V((S, DC), BF16),
        V((DM, NH, DH), BF16), V((DC, NH, DH), BF16), V((DC, NH, DH), BF16),
        V((NH, DM, DH), BF16), V((1, DM), BF16),
        V((S, DP), BF16), V((DM, 3 * DP), BF16), V((DM, DP), BF16),
        V((5, S + PADR, 128), F32), V((5, S + PADR, 128), F32), V((S, DP), BF16),
        V((2, S, DH), BF16), V((2, S, DH), BF16), V((2, S, DH), BF16),
        V((NH, S, DH), BF16), V((DM, S), BF16),
        pltpu.SemaphoreType.DMA((9,)), pltpu.SemaphoreType.DMA((8,)),
    ]
    out_t = pl.pallas_call(
        _kernel,
        out_shape=jax.ShapeDtypeStruct((1, DM, S), BF16),
        in_specs=[pl.BlockSpec(memory_space=pltpu.HBM)] * len(args),
        out_specs=pl.BlockSpec(memory_space=pltpu.HBM),
        scratch_shapes=scratch,
        compiler_params=pltpu.CompilerParams(vmem_limit_bytes=110 * 1024 * 1024),
    )(*args)
    return jnp.swapaxes(out_t, 1, 2)
```

```python
import functools
import math
import jax
import jax.numpy as jnp
from jax import lax
import jax.experimental.pallas as pl
import jax.experimental.pallas.tpu as pltpu

F32 = jnp.float32
BF16 = jnp.bfloat16
S, DM, NH, DH, DC = 2048, 576, 32, 128, 512
HA, DA, WIN, DIL = 32, 18, 8, 2
DP = 640
PADR = 16
BQ = 1024
RA = 256
TN = (((0,), (0,)), ((), ()))
NT = (((1,), (1,)), ((), ()))


def _dot(a, b):
    return jnp.dot(a, b, preferred_element_type=F32)


def _perm(n_in, off, transposed=False):
    shp = (DP, n_in) if transposed else (n_in, DP)
    src = lax.broadcasted_iota(jnp.int32, shp, 1 if transposed else 0)
    dst = lax.broadcasted_iota(jnp.int32, shp, 0 if transposed else 1)
    d = dst >> 5
    h = dst & 31
    return jnp.where((src == off + h * DA + d) & (d < DA), 1.0, 0.0).astype(BF16)


def _unpack(w):
    lo = lax.bitcast_convert_type(w << 16, F32).astype(BF16)
    hi = lax.bitcast_convert_type(w & jnp.uint32(0xFFFF0000), F32).astype(BF16)
    return lo, hi


def _kernel(x_h, wqkv_h, awo_h, c_h, wq_h, wuk_h, wuv_h, wo_h, gw_h, out_h,
            xt_v, wqkv_v, awo_v, c_v, wq_v, wuk_v, wuv_v, wo_v, gw_v,
            x_v, wa_p, awo_p, ka, va, oa, q_s, k_s, v_s, ctx, out_v, sems, osem):
    srcs = (x_h.at[0], wqkv_h, gw_h, awo_h, c_h.at[0], wq_h, wuk_h, wuv_h, wo_h)
    dsts = (xt_v.at[0:DM], wqkv_v, gw_v, awo_v, c_v, wq_v, wuk_v, wuv_v, wo_v)
    cps = [pltpu.make_async_copy(s, d, sems.at[i]) for i, (s, d) in enumerate(zip(srcs, dsts))]
    cps[1].start()
    cps[0].start()

    cps[1].wait()
    for p, (st, wd) in enumerate(((0, 640), (512, 640), (1152, 576))):
        wa_p[:, p * DP:(p + 1) * DP] = _dot(
            wqkv_v[:, st:st + wd], _perm(wd, p * DM - st)).astype(BF16)
    for t in range(5):
        ka[t, 0:PADR, :] = jnp.zeros((PADR, 128), F32)
        va[t, 0:PADR, :] = jnp.zeros((PADR, 128), F32)
    xt_v[DM:DP, :] = jnp.zeros((DP - DM, S), BF16)
    cps[0].wait()
    for i in (3, 4, 5, 6, 7, 2, 8):
        cps[i].start()

    def a_body(r, carry):
        r0 = pl.multiple_of(r * RA, RA)
        x_v[pl.ds(r0, RA), :] = xt_v[:, pl.ds(r0, RA)].T
        qkv = _dot(x_v[pl.ds(r0, RA), 0:DM], wa_p[...])
        for t in range(5):
            ka[t, pl.ds(r0 + PADR, RA), :] = qkv[:, DP + t * 128:DP + (t + 1) * 128]
            va[t, pl.ds(r0 + PADR, RA), :] = qkv[:, 2 * DP + t * 128:2 * DP + (t + 1) * 128]
        q = qkv[:, :DP] * (DA ** -0.5)
        pos = r0 + lax.broadcasted_iota(jnp.int32, (RA, 128), 0)
        lg = []
        for w in range(WIN):
            st = r0 + PADR - w * DIL
            acc = q[:, 0:128] * ka[0, pl.ds(st, RA), :]
            for t in range(1, 5):
                acc = acc + q[:, t * 128:(t + 1) * 128] * ka[t, pl.ds(st, RA), :]
            acc = acc + pltpu.roll(acc, 64, 1)
            acc = acc + pltpu.roll(acc, 32, 1)
            if w:
                acc = jnp.where(pos >= w * DIL, acc, -1e9)
            lg.append(acc)
        m = lg[0]
        for w in range(1, WIN):
            m = jnp.maximum(m, lg[w])
        e = [jnp.exp(l - m) for l in lg]
        den = e[0]
        for w in range(1, WIN):
            den = den + e[w]
        inv = 1.0 / den
        for t in range(5):
            o = e[0] * va[t, pl.ds(r0 + PADR, RA), :]
            for w in range(1, WIN):
                o = o + e[w] * va[t, pl.ds(r0 + PADR - w * DIL, RA), :]
            oa[pl.ds(r0, RA), t * 128:(t + 1) * 128] = (o * inv).astype(BF16)
        return carry

    lax.fori_loop(0, S // RA, a_body, 0)
    cps[3].wait()
    awo_p[...] = lax.dot_general(awo_v[...], _perm(DM, 0), TN, preferred_element_type=F32).astype(BF16)

    for i in (4, 5, 6, 7):
        cps[i].wait()
    wq_u, wuk_u, wuv_u = (r.bitcast(jnp.uint32) for r in (wq_v, wuk_v, wuv_v))
    qscale = DH ** -0.5 * math.log2(math.e)

    def pair_body(j, carry):
        wq2 = jnp.concatenate(_unpack(wq_u[:, j, :]), axis=1)
        wkv = jnp.concatenate(_unpack(wuk_u[:, j, :]) + _unpack(wuv_u[:, j, :]), axis=1)
        for r in range(S // 512):
            rs = slice(r * 512, (r + 1) * 512)
            q2 = (_dot(x_v[rs, 0:DM], wq2) * qscale).astype(BF16)
            kv = _dot(c_v[rs, :], wkv).astype(BF16)
            for a in range(2):
                q_s[a, rs, :] = q2[:, a * 128:(a + 1) * 128]
                k_s[a, rs, :] = kv[:, a * 128:(a + 1) * 128]
                v_s[a, rs, :] = kv[:, 256 + a * 128:256 + (a + 1) * 128]

        def head_body(a, c2):
            tri = (lax.broadcasted_iota(jnp.int32, (128, 128), 1)
                   <= lax.broadcasted_iota(jnp.int32, (128, 128), 0))
            nu = BQ // 128
            for i in reversed(range(S // BQ)):
                lo, hi = i * BQ, (i + 1) * BQ
                q = q_s[a, lo:hi, :]
                st = [lax.dot_general(q[u * 128:], k_s[a, lo + u * 128:lo + (u + 1) * 128, :], NT,
                                      preferred_element_type=F32) for u in range(nu)]
                tl = [[st[u][(r - u) * 128:(r - u + 1) * 128] for u in range(r + 1)] for r in range(nu)]
                for r in range(nu):
                    tl[r][r] = jnp.where(tri, tl[r][r], -1e9)
                mx = jnp.concatenate([functools.reduce(jnp.maximum, t) for t in tl], axis=0)
                if i:
                    so = lax.dot_general(q, k_s[a, 0:lo, :], NT, preferred_element_type=F32)
                    for t in range(lo // 128):
                        mx = jnp.maximum(mx, so[:, t * 128:(t + 1) * 128])
                m = jnp.max(mx, axis=1, keepdims=True)
                pt = [[jnp.exp2(t - m[r * 128:(r + 1) * 128]) for t in tl[r]] for r in range(nu)]
                ls = jnp.concatenate([functools.reduce(jnp.add, t) for t in pt], axis=0)
                od = [_dot(jnp.concatenate([pt[r][u] for r in range(u, nu)], axis=0).astype(BF16),
                           v_s[a, lo + u * 128:lo + (u + 1) * 128, :]) for u in range(nu)]
                o = jnp.concatenate(
                    [functools.reduce(jnp.add, [od[u][(r - u) * 128:(r - u + 1) * 128] for u in range(r + 1)])
                     for r in range(nu)], axis=0)
                if i:
                    po = jnp.exp2(so - m)
                    for t in range(lo // 128):
                        ls = ls + po[:, t * 128:(t + 1) * 128]
                    o = o + _dot(po.astype(BF16), v_s[a, 0:lo, :])
                l = jnp.sum(ls, axis=1, keepdims=True)
                ctx[2 * j + a, lo:hi, :] = (o * (1.0 / l)).astype(BF16)
            return c2

        lax.fori_loop(0, 2, head_body, 0, unroll=True)
        return carry

    lax.fori_loop(0, NH // 2, pair_body, 0)

    cps[8].wait()
    cps[2].wait()
    RO = 256

    def out_cp(r):
        rs = pl.ds(pl.multiple_of(r * RO, RO), RO)
        return pltpu.make_async_copy(out_v.at[:, rs], out_h.at[0, :, rs], osem.at[r])

    def o_body(r, carry):
        rs = pl.ds(pl.multiple_of(r * RO, RO), RO)
        cc = jnp.concatenate([ctx[h, rs, :] for h in range(NH)], axis=1)
        wo = jnp.concatenate([wo_v[h] for h in range(NH)], axis=1)
        b = lax.dot_general(wo, cc, NT, preferred_element_type=F32)
        a = lax.dot_general(awo_p[...], oa[rs, :], NT, preferred_element_type=F32)
        z = _dot(jnp.broadcast_to(gw_v[...], (16, DM)), xt_v[0:DM, rs])[0:1]
        g = 1.0 / (1.0 + jnp.exp(-z))
        out_v[:, rs] = (g * a + (1.0 - g) * b).astype(BF16)
        out_cp(r).start()
        return carry

    lax.fori_loop(0, S // RO, o_body, 0)
    for r in range(S // RO):
        out_cp(r).wait()


@jax.jit
def pallas_gated_mix__sliding_local_dilated__compressed_kv_cla__prompt_kernel(
    A_x, A_wqkv, A_wo, B_x, B_c_kv, B_w_q, B_w_uk, B_w_uv, B_w_o, gate_w,
):
    del B_x
    args = (jnp.swapaxes(A_x, 1, 2), A_wqkv, A_wo, B_c_kv, B_w_q, B_w_uk, B_w_uv,
            jnp.swapaxes(B_w_o, 1, 2), gate_w.reshape(1, DM))
    V = pltpu.VMEM
    scratch = [
        V((DP, S), BF16), V((DM, 3 * DM), BF16), V((DM, DM), BF16), V((S, DC), BF16),
        V((DM, NH, DH), BF16), V((DC, NH, DH), BF16), V((DC, NH, DH), BF16),
        V((NH, DM, DH), BF16), V((1, DM), BF16),
        V((S, DP), BF16), V((DM, 3 * DP), BF16), V((DM, DP), BF16),
        V((5, S + PADR, 128), F32), V((5, S + PADR, 128), F32), V((S, DP), BF16),
        V((2, S, DH), BF16), V((2, S, DH), BF16), V((2, S, DH), BF16),
        V((NH, S, DH), BF16), V((DM, S), BF16),
        pltpu.SemaphoreType.DMA((9,)), pltpu.SemaphoreType.DMA((8,)),
    ]
    out_t = pl.pallas_call(
        _kernel,
        out_shape=jax.ShapeDtypeStruct((1, DM, S), BF16),
        in_specs=[pl.BlockSpec(memory_space=pltpu.HBM)] * len(args),
        out_specs=pl.BlockSpec(memory_space=pltpu.HBM),
        scratch_shapes=scratch,
        compiler_params=pltpu.CompilerParams(vmem_limit_bytes=110 * 1024 * 1024),
    )(*args)
    return jnp.swapaxes(out_t, 1, 2)
```
